```python
import os as _os
_os.environ.setdefault("JAX_PLATFORMS", "cpu")
import jax
import jax.numpy as jnp

def _softmax(x, axis=-1):
    return jax.nn.softmax(x, axis=axis)
def _gelu(x):
    return jax.nn.gelu(x, approximate=True)
def _silu(x):
    return jax.nn.silu(x)
def _sigmoid(x):
    return jax.nn.sigmoid(x)
def _layernorm(x, axis=-1, eps=1e-5):
    m = jnp.mean(x, axis=axis, keepdims=True)
    v = jnp.var(x, axis=axis, keepdims=True)
    return (x - m) / jnp.sqrt(v + eps)
def _scatter_add(tgt, idx, src, axis=0):
    return tgt.at[idx].add(src)
def _segment_sum(src, seg, n):
    return jax.ops.segment_sum(src, seg, n)
class _Rng:
    def __init__(self, key):
        self._k = key
    def _next(self):
        self._k, sub = jax.random.split(self._k)
        return sub
    def normal(self, shape):
        return jax.random.normal(self._next(), shape, dtype=jnp.bfloat16)
    def randint(self, lo, hi, shape):
        return jax.random.randint(self._next(), shape, lo, hi, dtype=jnp.int32)
    def uniform(self, shape, lo=0.0, hi=1.0):
        return jax.random.uniform(self._next(), shape, jnp.bfloat16, lo, hi)
    def permutation(self, n):
        return jax.random.permutation(self._next(), n)


kernel_name = 'gated_mix__mha_block__mixer_s_mlp__prompt'

def setup_inputs():
    _rng = _Rng(jax.random.key(int.from_bytes(__import__("os").urandom(4), "little")))
    _w = (lambda a: (lambda t: t.astype(jnp.bfloat16) if jnp.issubdtype(t.dtype, jnp.floating) else t)(jnp.asarray(a)))
    def _A_setup():
        B, S, D, H = 1, 2048, 512, 32
        return {
            "x": _w((lambda *s: _rng.normal(s) * 0.05)(B, S, D)),
            "wqkv": _w((lambda *s: _rng.normal(s) * 0.8)(D, 3 * D)),
            "wo": _w((lambda *s: _rng.normal(s) * 0.05)(D, D)),
        }
    _A_in = _A_setup()

    def _B_setup():
        B, S, D, F = 1, 2048, 512, 1792
        return {
            "x":  _w((lambda *s: _rng.normal(s) * 0.05)(B, S, D)),
            "w1": _w((lambda *s: _rng.normal(s) * 0.2)(D, D) * (D ** -0.5)),
            "w2": _w((lambda *s: _rng.normal(s) * 0.2)(D, D) * (D ** -0.5)),
            "w3": _w((lambda *s: _rng.normal(s) * 0.2)(D, F) * (D ** -0.5)),
            "w4": _w((lambda *s: _rng.normal(s) * 0.2)(F, D) * (F ** -0.5)),
        }
    _B_in = _B_setup()

    return {
        "A_x": _A_in["x"],
        "A_wqkv": _A_in["wqkv"],
        "A_wo": _A_in["wo"],
        "B_x": _B_in["x"],
        "B_w1": _B_in["w1"],
        "B_w2": _B_in["w2"],
        "B_w3": _B_in["w3"],
        "B_w4": _B_in["w4"],
        "gate_w": _w((lambda *s: _rng.normal(s) * 0.05)(512) * 16.0),
    }

def reference(A_x, A_wqkv, A_wo, B_x, B_w1, B_w2, B_w3, B_w4, gate_w):
    def _A_ref(x, wqkv, wo):
        B, S, D = x.shape
        H = 32
        Dh = D // H
        qkv = (lambda x, *d: x.transpose(*d))((x @ wqkv).reshape(B, S, 3, H, Dh), 2, 0, 3, 1, 4)
        q, k, v = qkv[0], qkv[1], qkv[2]
        scores = jnp.einsum("bhqd,bhkd->bhqk", q, k) * (Dh ** -0.5)
        p = _softmax(scores, axis=-1)
        o = jnp.einsum("bhqk,bhkd->bhqd", p, v)
        return (lambda x, *d: x.transpose(*d))(o, 0, 2, 1, 3).reshape(B, S, D) @ wo

    def _B_ref(x, w1, w2, w3, w4):
        B, S, D = x.shape
        h = _gelu(_layernorm(x, axis=-1) @ w1)
        c = D // 4
        g0 = jnp.pad(h[:, :, 0*c:1*c], ((0, 0), (1, 0), (0, 0)))[:, :S, :]
        g1 = jnp.pad(h[:, :, 1*c:2*c], ((0, 0), (0, 1), (0, 0)))[:, 1:, :]
        g2 = jnp.pad(h[:, :, 2*c:3*c], ((0, 0), (2, 0), (0, 0)))[:, :S, :]
        g3 = jnp.pad(h[:, :, 3*c:   ], ((0, 0), (0, 2), (0, 0)))[:, 2:, :]
        hs = jnp.concatenate([g0, g1, g2, g3], axis=-1) @ w2
        x1 = x + hs
        h2 = _gelu(_layernorm(x1, axis=-1) @ w3) @ w4
        return x1 + h2

    x = A_x
    g = _sigmoid((x * gate_w).sum(-1, keepdims=True))
    a = _A_ref(x, A_wqkv, A_wo)
    b = _B_ref(x, B_w1, B_w2, B_w3, B_w4)
    return g * a + (1 - g) * b
```

```python
import functools
import math

import jax
import jax.numpy as jnp
import jax.experimental.pallas as pl
import jax.experimental.pallas.tpu as pltpu

_H = 32
_QT = 512
_KC = 128
_LAG = 2
_VK = 16
_DL = 1
_RT = 256
_OT = 512
_OS = 512
_PAD = 8

_L_MIN = 2.0 ** -40
_L_MAX = 2.0 ** 40
_A_MAX = 2.0 ** 126

_F32 = jnp.float32
_BF16 = jnp.bfloat16


def _layernorm(x):
    m = jnp.mean(x, axis=-1, keepdims=True)
    d = x - m
    v = jnp.mean(d * d, axis=-1, keepdims=True)
    return d * jax.lax.rsqrt(v + 1e-5)


def _gelu(x):
    c = math.sqrt(2.0 / math.pi)
    hx = 0.5 * x
    return hx + hx * jnp.tanh(x * (c + (c * 0.044715) * (x * x)))


def _dot(a, b):
    return jnp.dot(a, b, preferred_element_type=_F32)


def _kernel(xa_hbm, wqkv_hbm, wo_hbm, w1_hbm, w2_hbm, w3_hbm, w4_hbm,
            gw_ref, out_hbm,
            xa, wqkv, wo, w1, w2, w3, w4,
            wqvt, kk, kb, qt, vt, ot, bad_buf, p_buf, c_buf, s_buf, hbuf, obuf,
            ok_ref, sems, osems):
    S, D = xa.shape
    DH = D // _H
    HPG = 128 // DH
    NQ = S // _QT
    NC = S // _KC
    NR = S // _RT
    C = D // 4
    MG = (_KC - _VK) // 16

    def x_rows(r0, r1):
        rows = pl.ds(r0 * _RT, (r1 - r0) * _RT)
        return xa_hbm.at[rows], xa.at[rows]

    def w_cols(i):
        cols = pl.ds(i * D, D)
        return wqkv_hbm.at[:, cols], wqkv.at[:, cols]

    pairs = dict(
        x0=x_rows(0, 2), x1=x_rows(2, 4), x2=x_rows(4, NR),
        wq=w_cols(0), wk=w_cols(1), wv=w_cols(2), w1=(w1_hbm, w1),
        w2=(w2_hbm, w2), w3=(w3_hbm, w3), w4=(w4_hbm, w4), wo=(wo_hbm, wo))
    copies = {name: pltpu.make_async_copy(src, dst, sems.at[i])
              for i, (name, (src, dst)) in enumerate(pairs.items())}

    def start(*names):
        for name in names:
            copies[name].start()

    def wait(*names):
        for name in names:
            copies[name].wait()

    start("x0", "wk")
    hbuf[0:_PAD, :] = jnp.zeros((_PAD, D), _F32)
    hbuf[_PAD + S:_PAD + S + _PAD, :] = jnp.zeros((_PAD, D), _F32)
    p_buf[...] = jnp.zeros(p_buf.shape, _BF16)
    c_buf[...] = jnp.zeros(c_buf.shape, _F32)
    bad_buf[...] = jnp.zeros(bad_buf.shape, _F32)
    ok_ref[0] = 0
    qscale = (DH ** -0.5) * math.log2(math.e)

    def norm(r):
        return _layernorm(xa[r * _RT:(r + 1) * _RT, :].astype(_F32)).astype(_BF16)

    def proj_h(r, xn):
        hbuf[_PAD + r * _RT:_PAD + (r + 1) * _RT, :] = _gelu(_dot(xn, w1[...]))

    def proj_k(r):
        rows = slice(r * _RT, (r + 1) * _RT)
        k = _dot(xa[rows, :], wqkv[:, D:2 * D]).astype(_BF16)
        k = pltpu.bitcast(k, jnp.int32)
        for h in range(_H):
            g, j = divmod(h, HPG)
            kg = k[:, g * 128:(g + 1) * 128]
            kk[h, r * _RT // 2:(r + 1) * _RT // 2, :] = (
                pltpu.roll(kg, 128 - j * DH, 1) if j else kg)

    def proj_qv(r):
        rows = slice(r * _RT, (r + 1) * _RT)
        qv = jax.lax.dot_general(wqvt[...], xa[rows, :], (((1,), (1,)), ((), ())),
                                 preferred_element_type=_F32)
        qt[:, rows] = (qv[0:D] * qscale).astype(_BF16)
        vt[:, rows] = qv[D:2 * D].astype(_BF16)

    wait("x0", "wk")
    start("x1", "w1")
    proj_k(0)
    proj_k(1)
    xn0, xn1 = norm(0), norm(1)
    wait("x1", "w1")
    start("x2", "wq", "wv")
    proj_h(0, xn0)
    proj_h(1, xn1)
    for r in range(2, 4):
        proj_h(r, norm(r))
        proj_k(r)
    wait("x2", "wq", "wv")
    start("w2", "w3", "w4", "wo")
    proj_k(4)
    wqvt[0:D, :] = wqkv[:, 0:D].T
    wqvt[D:2 * D, :] = wqkv[:, 2 * D:3 * D].T
    for r in range(4, NR):
        proj_h(r, norm(r))
        if r > 4:
            proj_k(r)
        proj_qv(r - 4)
        proj_qv(r)

    def head_rows(h):
        return pl.ds(pl.multiple_of(h * DH, DH), DH)

    def half_rows(r0, n):
        start = r0 // 2
        if not isinstance(start, int):
            start = pl.multiple_of(start, 8)
        return pl.ds(start, n // 2)

    def k_rows(h, r0, n):
        return pltpu.bitcast(kk[h, half_rows(r0, n), :], _BF16)[:, :DH]

    def spread_keys(h, c):
        k = k_rows(h, c * _KC, _VK).astype(_F32)
        for d in range(DH):
            kb[c, d] = jnp.broadcast_to(k[:, d:d + 1], (_VK, 128))

    for c in range(NC):
        spread_keys(0, c)

    def finish(h, j, acc, l):
        l = jnp.sum(l, axis=0, keepdims=True)
        ot[head_rows(h), j * _QT:(j + 1) * _QT] = (acc * (1.0 / l)).astype(_BF16)
        ok_l = jnp.logical_and(l >= _L_MIN, l <= _L_MAX)
        bad = jnp.where(jnp.abs(acc) <= _A_MAX, jnp.where(ok_l, 0.0, 1.0), 1.0)
        bad = jnp.maximum(bad[0:8], bad[8:16])
        return functools.reduce(
            jnp.maximum, [bad[:, i * 128:(i + 1) * 128] for i in range(_QT // 128)])

    def fast_body(it, _):
        n = NQ * NC
        ps = {t: p_buf[t + _LAG] for t in range(-_LAG, 0)}
        acc = c_buf[0:DH]
        lprev = c_buf[DH:DH + 8]
        never = ok_ref[0] + it < 0
        marks = [None] * (_DL * MG)
        for t in range(n):
            tile, c = divmod(t, NC)
            u, j = divmod(tile, NQ)
            h = it + u
            if c == 0:
                if t:
                    lprev = l
                q = qt[head_rows(h), j * _QT:(j + 1) * _QT]
                qf = q.astype(_F32)
                l = jnp.zeros((8, _QT), _F32)
            sv = None
            for d in range(DH):
                kd = kb[c, d]
                r = d * MG // DH
                if marks[r] is not None and (d == 0 or (d - 1) * MG // DH != r):
                    kd = jnp.concatenate(
                        [jnp.where(never, marks[r], kd[i:i + 8])
                         for i in range(0, _VK, 8)], axis=0)
                term = jnp.concatenate([kd] * (_QT // 128), axis=1) * qf[d:d + 1, :]
                sv = term if sv is None else sv + term
            if j == NQ - 1:
                spread_keys(jnp.minimum(h + 1, _H - 1), c)
            s = _dot(k_rows(h, c * _KC + _VK, _KC - _VK), q)
            p = jnp.exp2(jnp.concatenate([sv, s], axis=0))
            marks = marks[MG:]
            for r in range(_KC // 8):
                l = l + p[8 * r:8 * r + 8]
                if r < 2 * MG and r % 2 == 1:
                    i = _QT // 128 - 1
                    marks.append(l[:, i * 128:(i + 1) * 128])
            ps[t] = p.astype(_BF16)
            tile, c = divmod(t - _LAG, NC)
            u, j = divmod(tile, NQ)
            h = it + u
            hc = jnp.maximum(h, 0)
            if c == 0:
                acc = jnp.zeros((DH, _QT), _F32)
            acc = acc + _dot(vt[head_rows(hc), c * _KC:(c + 1) * _KC], ps.pop(t - _LAG))
            if c == NC - 1:
                bad = finish(hc, j, acc, lprev)
                if tile >= 0 and j == 0:
                    bad_buf[h + 1] = bad
                else:
                    bad_buf[h + 1] = jnp.maximum(bad_buf[h + 1], bad)
        c_buf[0:DH] = acc
        c_buf[DH:DH + 8] = l
        for t in range(_LAG):
            p_buf[t] = ps[n - _LAG + t]
        return 0

    jax.lax.fori_loop(0, _H, fast_body, 0)
    acc = c_buf[0:DH]
    for t in range(_LAG):
        c0 = (NC - _LAG + t) * _KC
        acc = acc + _dot(vt[D - DH:D, c0:c0 + _KC], p_buf[t])
    bad_buf[_H] = jnp.maximum(
        bad_buf[_H], finish(_H - 1, NQ - 1, acc, c_buf[DH:DH + 8]))

    @pl.when(jnp.max(bad_buf[1:_H + 1].max(0)) > 0.0)
    def _():
        def head(h, _):
            @pl.when(jnp.max(bad_buf[h + 1]) > 0.0)
            def _():
                def tile(j, _):
                    cols = pl.ds(pl.multiple_of(j * _QT, _QT), _QT)
                    q = qt[head_rows(h), cols]

                    def scores(c, m):
                        rows = pl.ds(pl.multiple_of(c * _KC, _KC), _KC)
                        s = _dot(k_rows(h, c * _KC, _KC), q)
                        s_buf[rows, :] = s
                        return jnp.maximum(m, s.reshape(_KC // 8, 8, _QT).max(0))

                    m = jax.lax.fori_loop(
                        0, NC, scores, jnp.full((8, _QT), -jnp.inf, _F32))
                    m = jnp.max(m, axis=0, keepdims=True)

                    def pv(c, carry):
                        acc, l = carry
                        rows = pl.ds(pl.multiple_of(c * _KC, _KC), _KC)
                        p = jnp.exp2(s_buf[rows, :] - m)
                        v = vt[head_rows(h), rows]
                        return (acc + _dot(v, p.astype(_BF16)),
                                l + p.reshape(_KC // 8, 8, _QT).sum(0))

                    acc, l = jax.lax.fori_loop(
                        0, NC, pv,
                        (jnp.zeros((DH, _QT), _F32), jnp.zeros((8, _QT), _F32)))
                    l = jnp.sum(l, axis=0, keepdims=True)
                    ot[head_rows(h), cols] = (acc / l).astype(_BF16)
                    return 0

                jax.lax.fori_loop(0, NQ, tile, 0)
            return 0

        jax.lax.fori_loop(0, _H, head, 0)

    wait("w2", "w3", "w4", "wo")

    def out_copy(r, i):
        return pltpu.make_async_copy(
            obuf.at[r, i], out_hbm.at[pl.ds(r * _OT + i * _OS, _OS)], osems.at[r, i])

    def o_body(r, _):
        for i in range(_OT // _OS):
            r0 = pl.multiple_of(r * _OT + i * _OS, _OS)
            n = _OS + 2 * _PAD
            parts = []
            for gi, sh in enumerate((1, -1, 2, -2)):
                hh = hbuf[pl.ds(r0, n), gi * C:(gi + 1) * C]
                parts.append(
                    pltpu.roll(hh, sh % n, 0)[_PAD:_PAD + _OS].astype(_BF16))
            hs = _dot(jnp.concatenate(parts, axis=-1), w2[...])
            x = xa[pl.ds(r0, _OS), :].astype(_F32)
            x1 = x + hs
            a = _dot(ot[:, pl.ds(r0, _OS)].T, wo[...])
            t = _gelu(_dot(_layernorm(x1).astype(_BF16), w3[...])).astype(_BF16)
            b = x1 + _dot(t, w4[...])
            gate = jax.nn.sigmoid(jnp.sum(
                x * gw_ref[...].astype(_F32).reshape(1, D), axis=-1, keepdims=True))
            obuf[r, i] = (gate * a + (1.0 - gate) * b).astype(_BF16)
        for i in range(_OT // _OS):
            out_copy(r, i).start()
        return 0

    jax.lax.fori_loop(0, S // _OT, o_body, 0)
    for r in range(S // _OT):
        for i in range(_OT // _OS):
            out_copy(r, i).wait()


@jax.jit
def pallas_gated_mix__mha_block__mixer_s_mlp__prompt_kernel(
    A_x: jax.Array,
    A_wqkv: jax.Array,
    A_wo: jax.Array,
    B_x: jax.Array,
    B_w1: jax.Array,
    B_w2: jax.Array,
    B_w3: jax.Array,
    B_w4: jax.Array,
    gate_w: jax.Array,
):
    del B_x
    B, S, D = A_x.shape
    assert B == 1
    F = B_w3.shape[1]
    DH = D // _H
    hbm = pl.BlockSpec(memory_space=pl.ANY)
    vmem = pl.BlockSpec(memory_space=pltpu.VMEM)
    out = pl.pallas_call(
        _kernel,
        in_specs=[hbm] * 7 + [vmem],
        out_specs=hbm,
        out_shape=jax.ShapeDtypeStruct((S, D), A_x.dtype),
        scratch_shapes=[
            pltpu.VMEM((S, D), _BF16),
            pltpu.VMEM((D, 3 * D), _BF16),
            pltpu.VMEM((D, D), _BF16),
            pltpu.VMEM((D, D), _BF16),
            pltpu.VMEM((D, D), _BF16),
            pltpu.VMEM((D, F), _BF16),
            pltpu.VMEM((F, D), _BF16),
            pltpu.VMEM((2 * D, D), _BF16),
            pltpu.VMEM((_H, S // 2, 128), jnp.int32),
            pltpu.VMEM((S // _KC, DH, _VK, 128), _F32),
            pltpu.VMEM((D, S), _BF16),
            pltpu.VMEM((D, S), _BF16),
            pltpu.VMEM((D, S), _BF16),
            pltpu.VMEM((_H + 1, 8, 128), _F32),
            pltpu.VMEM((_LAG, _KC, _QT), _BF16),
            pltpu.VMEM((DH + 8, _QT), _F32),
            pltpu.VMEM((S, _QT), _F32),
            pltpu.VMEM((S + 2 * _PAD, D), _F32),
            pltpu.VMEM((S // _OT, _OT // _OS, _OS, D), _BF16),
            pltpu.SMEM((1,), jnp.int32),
            pltpu.SemaphoreType.DMA((11,)),
            pltpu.SemaphoreType.DMA((S // _OT, _OT // _OS)),
        ],
        compiler_params=pltpu.CompilerParams(vmem_limit_bytes=110 * 1024 * 1024),
    )(A_x.reshape(S, D), A_wqkv, A_wo, B_w1, B_w2, B_w3, B_w4, gate_w)
    return out.reshape(B, S, D)
```
